```python
import os as _os
_os.environ.setdefault("JAX_PLATFORMS", "cpu")
import jax
import jax.numpy as jnp

def _softmax(x, axis=-1):
    return jax.nn.softmax(x, axis=axis)
def _gelu(x):
    return jax.nn.gelu(x, approximate=True)
def _silu(x):
    return jax.nn.silu(x)
def _sigmoid(x):
    return jax.nn.sigmoid(x)
def _layernorm(x, axis=-1, eps=1e-5):
    m = jnp.mean(x, axis=axis, keepdims=True)
    v = jnp.var(x, axis=axis, keepdims=True)
    return (x - m) / jnp.sqrt(v + eps)
def _scatter_add(tgt, idx, src, axis=0):
    return tgt.at[idx].add(src)
def _segment_sum(src, seg, n):
    return jax.ops.segment_sum(src, seg, n)
class _Rng:
    def __init__(self, key):
        self._k = key
    def _next(self):
        self._k, sub = jax.random.split(self._k)
        return sub
    def normal(self, shape):
        return jax.random.normal(self._next(), shape, dtype=jnp.bfloat16)
    def randint(self, lo, hi, shape):
        return jax.random.randint(self._next(), shape, lo, hi, dtype=jnp.int32)
    def uniform(self, shape, lo=0.0, hi=1.0):
        return jax.random.uniform(self._next(), shape, jnp.bfloat16, lo, hi)
    def permutation(self, n):
        return jax.random.permutation(self._next(), n)


kernel_name = 'standalone__dcn_v2_cross__recsys'

def setup_inputs():
    _rng = _Rng(jax.random.key(int.from_bytes(__import__("os").urandom(4), "little")))
    _w = (lambda a: (lambda t: t.astype(jnp.bfloat16) if jnp.issubdtype(t.dtype, jnp.floating) else t)(jnp.asarray(a)))
    B, F, D, L = 4096, 26, 128, 6
    Din = min(F * D, 1024)
    return {
        "x0": _w((lambda *s: _rng.normal(s) * 0.05)(B, Din)),
        "ws": _w((lambda *s: _rng.normal(s) * 0.05)(L, Din, Din)),
        "bs": _w((lambda *s: _rng.normal(s) * 0.05)(L, Din)),
    }

def reference(x0, ws, bs):
    x = x0
    for l in range(ws.shape[0]):
        x = x0 * (x @ ws[l] + bs[l]) + x
    return x
```

```python
import jax
import jax.numpy as jnp
import jax.experimental.pallas as pl
import jax.experimental.pallas.tpu as pltpu

TM = 512
OUT_CHUNKS = (384, 384, 128, 128)
PLAN = ([[('x',0,384,0,512),('w',0,512,0,384)], [(0,384,0,512,0,384)]],
        [[('x',0,384,512,1024),('w',512,1024,0,384)], [(0,384,512,1024,0,384)]],
        [[('w',0,1024,384,640)], [(0,384,0,1024,384,640)]],
        [[('w',0,1024,640,1024),('x',384,512,0,1024)], [(0,512,0,1024,640,1024),(384,512,0,1024,0,640)]])

f32, bf16 = jnp.float32, jnp.bfloat16
ncp = sum(len(s[0]) for s in PLAN)

def kern(x_hbm, w_hbm, b_hbm, o_hbm, xb, wb, bb, b32, ob, xs, acc, xsem, wsem, psem, bsem, osem):
    L, D = wb.shape[0], wb.shape[1]
    NT = xb.shape[0]
    def xcp(t):
        return pltpu.make_async_copy(x_hbm.at[pl.ds(t * TM, TM)], xb.at[t], xsem.at[t])
    def wcp(l):
        return pltpu.make_async_copy(w_hbm.at[l], wb.at[l], wsem.at[l])
    cps, n = [], 0
    for copies, _ in PLAN:
        cs = []
        for kind, r0, r1, c0, c1 in copies:
            r, c = pl.ds(r0, r1 - r0), pl.ds(c0, c1 - c0)
            if kind == 'x':
                cs.append(pltpu.make_async_copy(x_hbm.at[r, c], xb.at[0, r, c], psem.at[n]))
            else:
                cs.append(pltpu.make_async_copy(w_hbm.at[0, r, c], wb.at[0, r, c], psem.at[n]))
            n += 1
        cps.append(cs)
    cps.append([wcp(1)])
    bcp = pltpu.make_async_copy(b_hbm, bb, bsem)
    started = 0
    def start_upto(j):
        nonlocal started
        while started <= min(j, len(cps) - 1):
            for c in cps[started]: c.start()
            started += 1
    start_upto(0); bcp.start(); start_upto(1)
    for j, (_, dots) in enumerate(PLAN):
        if j == 0: bcp.wait()
        for c in cps[j]: c.wait()
        start_upto(j + 2)
        for r0, r1, k0, k1, c0, c1 in dots:
            y = jnp.dot(xb[0, r0:r1, k0:k1], wb[0, k0:k1, c0:c1], preferred_element_type=f32)
            y = y + (bb[0:1, c0:c1].astype(f32) if k0 == 0 else acc[r0:r1, c0:c1])
            if k1 < D:
                acc[r0:r1, c0:c1] = y
            else:
                x0f = xb[0, r0:r1, c0:c1].astype(f32)
                xs[r0:r1, c0:c1] = (x0f * y + x0f).astype(bf16)
    b32[...] = bb[...].astype(f32)

    def warm(l, carry):
        wcp(l).wait()
        @pl.when(l + 1 < L)
        def _():
            wcp(l + 1).start()
        xcp(l).start()
        x = xs[...]
        y = jnp.dot(x, wb[l], preferred_element_type=f32) + b32[pl.ds(l, 1), :]
        xs[...] = (xb[0].astype(f32) * y + x.astype(f32)).astype(bf16)
        return carry
    jax.lax.fori_loop(1, L, warm, 0)
    for t in range(L, NT):
        xcp(t).start()
    pltpu.make_async_copy(xs, o_hbm.at[pl.ds(0, TM)], osem).start()

    def main(t, carry):
        xcp(t).wait()
        x = xb[t]
        x0f = x.astype(f32)
        for l in range(L - 1):
            y = jnp.dot(x, wb[l], preferred_element_type=f32) + bb[l:l+1, :].astype(f32)
            x = (x0f * y + x.astype(f32)).astype(bf16)
        l = L - 1
        c0 = 0
        for w in OUT_CHUNKS:
            s = slice(c0, c0 + w); c0 += w
            y = jnp.dot(x, wb[l, :, s], preferred_element_type=f32) + bb[l:l+1, s].astype(f32)
            ob[t, :, s] = (x0f[:, s] * y + x[:, s].astype(f32)).astype(bf16)
            pltpu.make_async_copy(ob.at[t, :, s], o_hbm.at[pl.ds(t * TM, TM), s], osem).start()
        return carry
    jax.lax.fori_loop(1, NT, main, 0)
    pltpu.make_async_copy(o_hbm, o_hbm, osem).wait()

@jax.jit
def pallas_standalone__dcn_v2_cross__recsys_kernel(x0, ws, bs):
    B, D = x0.shape
    L = ws.shape[0]
    NT = B // TM
    assert B % TM == 0 and D == sum(OUT_CHUNKS) and 2 <= L <= NT
    any_ = pl.BlockSpec(memory_space=pl.ANY)
    return pl.pallas_call(
        kern,
        in_specs=[any_, any_, any_],
        out_specs=any_,
        out_shape=jax.ShapeDtypeStruct((B, D), jnp.bfloat16),
        scratch_shapes=[pltpu.VMEM((NT, TM, D), bf16), pltpu.VMEM((L, D, D), bf16), pltpu.VMEM((L, D), bf16), pltpu.VMEM((L, D), f32),
                        pltpu.VMEM((NT, TM, D), bf16), pltpu.VMEM((TM, D), bf16), pltpu.VMEM((TM, D), f32),
                        pltpu.SemaphoreType.DMA((NT,)), pltpu.SemaphoreType.DMA((L,)), pltpu.SemaphoreType.DMA((ncp,)),
                        pltpu.SemaphoreType.DMA(()), pltpu.SemaphoreType.DMA(())],
        compiler_params=pltpu.CompilerParams(vmem_limit_bytes=100 * 1024 * 1024),
    )(x0, ws, bs)
```
